```python
import jax
import jax.numpy as jnp

def _softmax(x, axis=-1):
    return jax.nn.softmax(x, axis=axis)

def _gelu(x):
    return jax.nn.gelu(x, approximate=True)

def _silu(x):
    return jax.nn.silu(x)

def _sigmoid(x):
    return jax.nn.sigmoid(x)

def _layernorm(x, axis=-1, eps=1e-05):
    m = jnp.mean(x, axis=axis, keepdims=True)
    v = jnp.var(x, axis=axis, keepdims=True)
    return (x - m) / jnp.sqrt(v + eps)

def _scatter_add(tgt, idx, src, axis=0):
    return tgt.at[idx].add(src)

def _segment_sum(src, seg, n):
    return jax.ops.segment_sum(src, seg, n)

class _Rng:

    def __init__(self, key):
        self._k = key

    def _next(self):
        self._k, sub = jax.random.split(self._k)
        return sub

    def normal(self, shape):
        return jax.random.normal(self._next(), shape, dtype=jnp.bfloat16)

    def randint(self, lo, hi, shape):
        return jax.random.randint(self._next(), shape, lo, hi, dtype=jnp.int32)

    def uniform(self, shape, lo=0.0, hi=1.0):
        return jax.random.uniform(self._next(), shape, jnp.bfloat16, lo, hi)

    def permutation(self, n):
        return jax.random.permutation(self._next(), n)
kernel_name = 'adaLN_cond__sliding_block_cached__glu_gated_glu__decode'

def setup_inputs():
    _rng = _Rng(jax.random.key(int.from_bytes(__import__("os").urandom(4), "little")))
    _w = lambda a: (lambda t: t.astype(jnp.bfloat16) if jnp.issubdtype(t.dtype, jnp.floating) else t)(jnp.asarray(a))

    def _A_setup():
        B, Sq, D = (8, 1, 512)
        Hq, Hkv, Sk, Dh = (32, 32, 4096, 128)
        assert Hq % Hkv == 0, (Hq, Hkv)
        return {'x': _w((lambda *s: _rng.normal(s) * 0.05)(B, Sq, D)), 'k_cache': _w((lambda *s: _rng.normal(s) * 0.05)(B, Hkv, Sk, Dh)), 'v_cache': _w((lambda *s: _rng.normal(s) * 0.05)(B, Hkv, Sk, Dh)), 'wq': _w((lambda *s: _rng.normal(s) * 0.05)(D, Hq * Dh) * D ** (-0.5)), 'wo': _w((lambda *s: _rng.normal(s) * 0.05)(Hq * Dh, D) * (Hq * Dh) ** (-0.5))}
    _A_in = _A_setup()

    def _B_setup():
        B, S, D, F = (8, 1, 512, 1376)
        return {'x': _w((lambda *s: _rng.normal(s) * 0.05)(B, S, D)), 'w_gate': _w((lambda *s: _rng.normal(s) * 0.05)(D, F)), 'w_up': _w((lambda *s: _rng.normal(s) * 0.05)(D, F)), 'w_down': _w((lambda *s: _rng.normal(s) * 0.05)(F, D))}
    _B_in = _B_setup()
    return {'A_x': _A_in['x'], 'A_k_cache': _A_in['k_cache'], 'A_v_cache': _A_in['v_cache'], 'A_wq': _A_in['wq'], 'A_wo': _A_in['wo'], 'B_x': _B_in['x'], 'B_w_gate': _B_in['w_gate'], 'B_w_up': _B_in['w_up'], 'B_w_down': _B_in['w_down'], 'c': _w((lambda *s: _rng.normal(s) * 0.05)(8, 512)), 'w_mod': _w((lambda *s: _rng.normal(s) * 0.05)(512, 6 * 512) * 512 ** (-0.5))}

def reference(A_x, A_k_cache, A_v_cache, A_wq, A_wo, B_x, B_w_gate, B_w_up, B_w_down, c, w_mod):

    def _A_ref(x, k_cache, v_cache, wq, wo):
        B, Sq, D = x.shape
        Hq, Dh = (32, 128)
        Hkv, Sk = (k_cache.shape[1], k_cache.shape[2])
        W = min(4096, max(256, Sk // 4))
        rep = Hq // Hkv
        q = (lambda x, *d: x.transpose(*d))((x @ wq).reshape(B, Sq, Hq, Dh), 0, 2, 1, 3)
        k = jnp.repeat(k_cache[:, :, Sk - W:, :], rep, axis=1)
        v = jnp.repeat(v_cache[:, :, Sk - W:, :], rep, axis=1)
        scores = jnp.einsum('bhqd,bhkd->bhqk', q, k) * Dh ** (-0.5)
        p = _softmax(scores, axis=-1)
        o = jnp.einsum('bhqk,bhkd->bhqd', p, v)
        return (lambda x, *d: x.transpose(*d))(o, 0, 2, 1, 3).reshape(B, Sq, Hq * Dh) @ wo

    def _B_ref(x, w_gate, w_up, w_down):
        g = jnp.einsum('bsd,df->bsf', x, w_gate)
        u = jnp.einsum('bsd,df->bsf', x, w_up)
        h = _sigmoid(g) * u
        return jnp.einsum('bsf,fd->bsd', h, w_down)
    x = A_x
    mod = (_silu(c) @ w_mod).reshape(c.shape[0], 6, 1, -1)
    sa, ca, ga, sb, cb, gb = (mod[:, 0].copy(), mod[:, 1].copy(), mod[:, 2].copy(), mod[:, 3].copy(), mod[:, 4].copy(), mod[:, 5].copy())
    h = _layernorm(x, axis=-1) * (1 + ca) + sa
    x = x + ga * _A_ref(h, A_k_cache, A_v_cache, A_wq, A_wo)
    h = _layernorm(x, axis=-1) * (1 + cb) + sb
    x = x + gb * _B_ref(h, B_w_gate, B_w_up, B_w_down)
    return x
```

```python
import functools
import jax
import jax.numpy as jnp
from jax import lax
import jax.experimental.pallas as pl
import jax.experimental.pallas.tpu as pltpu

B, D, H, DH, F = 8, 512, 32, 128, 1376
CH = 128
R = 32
NJ = 2
HG = H // NJ
NSTR = B * NJ
NS = 8
NSEM = 16
NT = (((1,), (1,)), ((), ()))
f32, bf16 = jnp.float32, jnp.bfloat16
cpy = pltpu.make_async_copy


def _ln(x):
    m = jnp.mean(x, axis=-1, keepdims=True)
    d = x - m
    v = jnp.mean(d * d, axis=-1, keepdims=True)
    return d * lax.rsqrt(v + 1e-5)


def _body(x_hbm, k_hbm, v_hbm, wq_hbm, wo_hbm, wg_hbm, wu_hbm, wd_hbm, c_hbm, wm_hbm,
          o_ref,
          kv, xs, cs, wm, wq, wo, wg, wu, wd, oacc, sbuf, pbuf, part, linv, qbuf, sems, wsems, xsem,
          *, S, W, LOOK, n0, compute, scopes):
    NCH = W // CH
    PPC = CH // R
    PPS = NCH * PPC
    assert PPS % NSEM == 0 and NCH % NS == 0 and LOOK <= NSEM and LOOK <= PPC * (NS - 2)
    import contextlib
    scope = (lambda n: jax.named_scope(n)) if scopes else (lambda n: contextlib.nullcontext())

    def rows_job(src, dst, r0, n0_, n, c0=None, nc=None):
        def sl(ref, a, m):
            if c0 is None:
                return ref.at[pl.ds(a, m), :]
            return ref.at[pl.ds(a, m), pl.ds(c0, nc)]
        return [(sl(src, r0, n0_), sl(dst, r0, n0_), 0), (sl(src, r0 + n0_, n - n0_), sl(dst, r0 + n0_, n - n0_), 1)]

    sjobs = [rows_job(wm_hbm, wm, 64 * j, 16, 64, 0, 2 * D) for j in range(D // 64)]
    n_moda = len(sjobs)
    sjobs += [[(wq_hbm.at[pl.ds(16 * j, 16), pl.ds(0, 512)], wq.at[pl.ds(16 * j, 16), pl.ds(0, 512)], 0),
               (wq_hbm.at[pl.ds(16 * j, 16), pl.ds(512, H * DH - 512)], wq.at[pl.ds(16 * j, 16), pl.ds(512, H * DH - 512)], 1)]
              for j in range(D // 16)]
    NSJ = len(sjobs)
    ejobs = [[(wm_hbm.at[pl.ds(32 * j, 16), pl.ds(2 * D, D)], wm.at[pl.ds(32 * j, 16), pl.ds(2 * D, D)], 0),
              (wm_hbm.at[pl.ds(32 * j, 16), pl.ds(3 * D, 3 * D)], wm.at[pl.ds(32 * j, 16), pl.ds(3 * D, 3 * D)], 1),
              (wm_hbm.at[pl.ds(32 * j + 16, 16), pl.ds(2 * D, 4 * D)], wm.at[pl.ds(32 * j + 16, 16), pl.ds(2 * D, 4 * D)], 1)]
             for j in range(D // 32)]
    n_modb = len(ejobs)
    ejobs += [rows_job(wo_hbm, wo, DH * j, 16, DH) for j in range(H)]
    fch = [(128 * j, min(128, F - 128 * j)) for j in range(-(-F // 128))]
    for f0, n in fch:
        ejobs += [rows_job(wg_hbm, wg, f0, 16, n), rows_job(wu_hbm, wu, f0, 16, n), rows_job(wd_hbm, wd, f0, 16, n)]
    NEJ = len(ejobs)

    def start_job(job, g):
        for src, dst, prio in sorted(job, key=lambda t: -t[2]):
            cpy(src, dst, wsems.at[g % NSEM]).start(priority=prio)

    def wait_job(job, g):
        for src, dst, prio in job:
            cpy(src, dst, wsems.at[g % NSEM]).wait()

    def start_piece(h, t, r):
        c, pc = divmod(r, PPC)
        rows = pl.ds(S - W + r * R, R)
        dst = pl.ds(pc * R, R)
        src = (k_hbm, v_hbm)[t]
        sem = sems.at[r % NSEM]
        cpy(src.at[pl.ds(n0, NSTR - n0), h, rows, :], kv.at[c % NS, pl.ds(n0, NSTR - n0), dst], sem).start(priority=1)
        cpy(src.at[pl.ds(0, n0), h, rows, :], kv.at[c % NS, pl.ds(0, n0), dst], sem).start(priority=0)

    def wait_piece(r):
        c, pc = divmod(r, PPC)
        dst = kv.at[c % NS, :, pl.ds(pc * R, R)]
        cpy(dst, dst, sems.at[r % NSEM]).wait()

    def pump_s(j):
        with scope(f"S{j:02d}"):
            wait_job(sjobs[j], j)
        j2 = j + LOOK
        if j2 < NSJ:
            start_job(sjobs[j2], j2)
        else:
            start_piece(0, 0, j2 - NSJ)

    def pump(h, t, r):
        wait_piece(r)
        r2 = r + LOOK
        if r2 < PPS:
            start_piece(h, t, r2)
        elif t == 0:
            start_piece(h, 1, r2 - PPS)
        else:
            @pl.when(h + 1 < HG)
            def _():
                start_piece(h + 1, 0, r2 - PPS)

            @pl.when(h + 1 == HG)
            def _():
                start_job(ejobs[r2 - PPS], r2 - PPS)

    def pump_e(j):
        with scope(f"E{j:02d}"):
            wait_job(ejobs[j], j)
        j2 = j + LOOK
        if j2 < NEJ:
            start_job(ejobs[j2], j2)

    row = lax.broadcasted_iota(jnp.int32, (B, DH), 0)
    scale = DH ** -0.5

    def qproj(h1, h, j):
        off = (h + j * HG) * DH
        if not isinstance(off, int):
            off = pl.multiple_of(off, DH)
        qbuf[j] = jnp.dot(h1, wq[:, pl.ds(off, DH)], preferred_element_type=f32)

    def qk4(c, u, prev):
        j, bh = divmod(u, 2)
        q = qbuf[j].astype(bf16)
        out = prev
        for b in range(4 * bh, 4 * bh + 4):
            sb = lax.dot_general(q, kv[c % NS, NJ * b + j], NT, preferred_element_type=f32)
            out = sb if out is None else jnp.where(row == b, sb, out)
        if bh == 1:
            sbuf[j, c] = out
            return None
        return out

    def pv4(c, u, acc):
        j, bh = divmod(u, 2)
        p = pbuf[j, c]
        for b in range(4 * bh, 4 * bh + 4):
            pb = jnp.where(row == b, p, 0.0).astype(bf16)
            d = jnp.dot(pb, kv[c % NS, NJ * b + j], preferred_element_type=f32)
            acc[j] = d if acc[j] is None else acc[j] + d

    def softmax_max():
        return [jnp.max(functools.reduce(jnp.maximum, [sbuf[j, c] for c in range(NCH)]), axis=-1, keepdims=True)
                for j in range(NJ)]

    def softmax_exp(m):
        for j in range(NJ):
            tot = None
            for c in range(NCH):
                p = jnp.exp((sbuf[j, c] - m[j]) * scale)
                pbuf[j, c] = p
                tot = p if tot is None else tot + p
            linv[j] = jnp.broadcast_to(1.0 / jnp.sum(tot, axis=-1, keepdims=True), (B, DH))

    def pv_last(u, acc, hprev):
        j, bh = divmod(u, 2)
        if bh == 0:
            acc[j] = part[j]
        pv4(NCH - 1, u, acc)
        if bh == 1:
            oacc[hprev + j * HG] = acc[j] * linv[j]

    cc = cpy(c_hbm, cs, xsem.at[0])
    cx = cpy(x_hbm, xs, xsem.at[1])
    cc.start(priority=0)
    cx.start(priority=0)
    for j in range(LOOK):
        start_job(sjobs[j], j)
    pbuf[...] = jnp.zeros_like(pbuf)
    part[...] = jnp.zeros_like(part)
    linv[...] = jnp.zeros_like(linv)
    kv[(NCH - 1) % NS] = jnp.zeros(kv.shape[1:], bf16)
    pump_s(0)
    with scope("cx"):
        cc.wait()
        cx.wait()
    cf = cs[...].astype(f32)
    sc = (cf * jax.nn.sigmoid(cf)).astype(bf16)
    x = xs[...].astype(f32)
    pump_s(1)
    lnx = _ln(x)
    for j in range(2, n_moda):
        pump_s(j)
    moda = jnp.dot(sc, wm[:, :2 * D], preferred_element_type=f32)
    pump_s(n_moda)
    h1 = (lnx * (1.0 + moda[:, D:]) + moda[:, :D]).astype(bf16)
    for j in range(n_moda + 1, NSJ):
        pump_s(j)

    def group(h, carry):
        hprev = jnp.where(h > 0, h - 1, H)
        acc = [None] * NJ
        st = None
        for r in range(PPS):
            pump(h, 0, r)
            if not compute:
                continue
            c, u = divmod(r, PPC)
            if c == 0:
                pv_last(u, acc, hprev)
                if u < NJ:
                    qproj(h1, h, u)
            else:
                st = qk4(c - 1, u, st)
        acc = [None] * NJ
        for r in range(PPS):
            pump(h, 1, r)
            if not compute:
                continue
            c, u = divmod(r, PPC)
            if c == 0:
                st = qk4(NCH - 1, u, st)
            elif c == 1:
                if u == 0:
                    m = softmax_max()
                elif u == 1:
                    softmax_exp(m)
                else:
                    pv4(0, 2 * (u - 2), acc)
                    pv4(0, 2 * (u - 2) + 1, acc)
            else:
                pv4(c - 1, u, acc)
        if compute:
            for j in range(NJ):
                part[j] = acc[j]
        return carry

    if not compute:
        oacc[...] = jnp.zeros_like(oacc)
    lax.fori_loop(0, HG, group, 0)

    acc = [None] * NJ
    modb = None
    for j in range(n_modb):
        pump_e(j)
        if j < PPC and compute:
            pv_last(j, acc, HG - 1)
        if j % 4 == 3:
            d = jnp.dot(sc[:, 32 * (j - 3):32 * (j + 1)], wm[pl.ds(32 * (j - 3), 128), 2 * D:], preferred_element_type=f32)
            modb = d if modb is None else modb + d
    attn = jnp.zeros((B, D), f32)
    for j in range(H):
        pump_e(n_modb + j)
        attn = attn + jnp.dot(oacc[j].astype(bf16), wo[pl.ds(DH * j, DH), :], preferred_element_type=f32)
    x1 = x + modb[:, 0:D] * attn
    h2 = (_ln(x1) * (1.0 + modb[:, 2 * D:3 * D]) + modb[:, D:2 * D]).astype(bf16)
    y = jnp.zeros((B, D), f32)
    g0 = n_modb + H
    for i, (f0, n) in enumerate(fch):
        pump_e(g0 + 3 * i)
        g = lax.dot_general(h2, wg[pl.ds(f0, n), :], NT, preferred_element_type=f32)
        pump_e(g0 + 3 * i + 1)
        u = lax.dot_general(h2, wu[pl.ds(f0, n), :], NT, preferred_element_type=f32)
        a = (jax.nn.sigmoid(g) * u).astype(bf16)
        pump_e(g0 + 3 * i + 2)
        y = y + jnp.dot(a, wd[pl.ds(f0, n), :], preferred_element_type=f32)
    o_ref[...] = (x1 + modb[:, 3 * D:] * y).astype(o_ref.dtype)


@jax.jit
def pallas_adaLN_cond__sliding_block_cached__glu_gated_glu__decode_kernel(
    A_x, A_k_cache, A_v_cache, A_wq, A_wo, B_x, B_w_gate, B_w_up, B_w_down, c, w_mod,
):
    del B_x
    S = A_k_cache.shape[2]
    W = min(4096, max(256, S // 4))
    hbm = pl.BlockSpec(memory_space=pltpu.HBM)
    out = pl.pallas_call(
        functools.partial(_body, S=S, W=W, LOOK=8, n0=2, compute=True, scopes=False),
        out_shape=jax.ShapeDtypeStruct((B, D), A_x.dtype),
        in_specs=[hbm] * 10,
        out_specs=pl.BlockSpec(memory_space=pltpu.VMEM),
        scratch_shapes=[
            pltpu.VMEM((NS, NSTR, CH, DH), bf16),
            pltpu.VMEM((B, D), bf16),
            pltpu.VMEM((B, D), bf16),
            pltpu.VMEM((D, 6 * D), bf16),
            pltpu.VMEM((D, H * DH), bf16),
            pltpu.VMEM((H * DH, D), bf16),
            pltpu.VMEM((F, D), bf16),
            pltpu.VMEM((F, D), bf16),
            pltpu.VMEM((F, D), bf16),
            pltpu.VMEM((H + HG + 1, B, DH), f32),
            pltpu.VMEM((NJ, W // CH, B, DH), f32),
            pltpu.VMEM((NJ, W // CH, B, DH), f32),
            pltpu.VMEM((NJ, B, DH), f32),
            pltpu.VMEM((NJ, B, DH), f32),
            pltpu.VMEM((NJ, B, DH), f32),
            pltpu.SemaphoreType.DMA((NSEM,)),
            pltpu.SemaphoreType.DMA((NSEM,)),
            pltpu.SemaphoreType.DMA((2,)),
        ],
        compiler_params=pltpu.CompilerParams(
            vmem_limit_bytes=64 * 1024 * 1024, disable_bounds_checks=True),
    )(A_x.reshape(B, D), A_k_cache.reshape(NSTR, HG, S, DH), A_v_cache.reshape(NSTR, HG, S, DH),
      A_wq, A_wo, B_w_gate.T, B_w_up.T, B_w_down, c, w_mod)
    return out.reshape(B, 1, D)
```

```python
import functools
import jax
import jax.numpy as jnp
from jax import lax
import jax.experimental.pallas as pl
import jax.experimental.pallas.tpu as pltpu

B, D, H, DH, F = 8, 512, 32, 128, 1376
CH = 128
R = 32
NJ = 2
HG = H // NJ
NSTR = B * NJ
NS = 8
NSEM = 16
NW = 8
NT = (((1,), (1,)), ((), ()))
f32, bf16 = jnp.float32, jnp.bfloat16
cpy = pltpu.make_async_copy


def _ln(x):
    m = jnp.mean(x, axis=-1, keepdims=True)
    d = x - m
    v = jnp.mean(d * d, axis=-1, keepdims=True)
    return d * lax.rsqrt(v + 1e-5)


def _body(x_hbm, k_hbm, v_hbm, wq_hbm, wo_hbm, wg_hbm, wu_hbm, wd_hbm, c_hbm, wm_hbm,
          o_ref,
          kv, xs, cs, wm, wq, wo, wg, wu, wd, oacc, sbuf, pbuf, part, linv, qbuf, sems, wsems, xsem,
          *, S, W, LOOK, n0, compute, scopes):
    NCH = W // CH
    PPC = CH // R
    PPS = NCH * PPC
    assert PPS % NSEM == 0 and NCH % NS == 0 and LOOK <= NSEM and LOOK <= PPC * (NS - 2)
    import contextlib
    scope = (lambda n: jax.named_scope(n)) if scopes else (lambda n: contextlib.nullcontext())

    def rows_job(src, dst, r0, n0_, n, c0=None, nc=None):
        def sl(ref, a, m):
            if c0 is None:
                return ref.at[pl.ds(a, m), :]
            return ref.at[pl.ds(a, m), pl.ds(c0, nc)]
        return [(sl(src, r0, n0_), sl(dst, r0, n0_), 0), (sl(src, r0 + n0_, n - n0_), sl(dst, r0 + n0_, n - n0_), 1)]

    def strm_job(src, dst, r0, nr, c0, nc):
        def sl(ref, a, n):
            return ref.at[pl.ds(a, n), pl.ds(r0, nr), pl.ds(c0, nc)]
        return [(sl(src, 0, 1), sl(dst, 0, 1), 0), (sl(src, 1, NW - 1), sl(dst, 1, NW - 1), 1)]

    def wm_jobs(cb):
        return [strm_job(wm_hbm, wm, 8 * j, 8, 2 * D * cb, 2 * D) for j in range(D // NW // 8)]

    sjobs = wm_jobs(0)
    n_moda = len(sjobs)
    sjobs += [strm_job(wq_hbm, wq, 8 * rb, 8, 1024 * cb, 1024) for rb in range(D // NW // 8) for cb in range(H * DH // 1024)]
    NSJ = len(sjobs)
    ejobs = [strm_job(wo_hbm, wo, 16 * j, 16, 0, D) for j in range(H * DH // NW // 16)]
    n_wo = len(ejobs)
    ejobs += wm_jobs(1) + wm_jobs(2)
    g0 = len(ejobs)
    n_m1 = (g0 - n_wo) // 2
    fch = [(128 * j, min(128, F - 128 * j)) for j in range(-(-F // 128))]
    for f0, n in fch:
        ejobs += [rows_job(wg_hbm, wg, f0, 16, n), rows_job(wu_hbm, wu, f0, 16, n), rows_job(wd_hbm, wd, f0, 16, n)]
    NEJ = len(ejobs)

    def start_job(job, g):
        for src, dst, prio in sorted(job, key=lambda t: -t[2]):
            cpy(src, dst, wsems.at[g % NSEM]).start(priority=prio)

    def wait_job(job, g):
        for src, dst, prio in job:
            cpy(src, dst, wsems.at[g % NSEM]).wait()

    def start_piece(h, t, r):
        c, pc = divmod(r, PPC)
        rows = pl.ds(S - W + r * R, R)
        dst = pl.ds(pc * R, R)
        src = (k_hbm, v_hbm)[t]
        sem = sems.at[r % NSEM]
        cpy(src.at[pl.ds(n0, NSTR - n0), h, rows, :], kv.at[c % NS, pl.ds(n0, NSTR - n0), dst], sem).start(priority=1)
        cpy(src.at[pl.ds(0, n0), h, rows, :], kv.at[c % NS, pl.ds(0, n0), dst], sem).start(priority=0)

    def wait_piece(r):
        c, pc = divmod(r, PPC)
        dst = kv.at[c % NS, :, pl.ds(pc * R, R)]
        cpy(dst, dst, sems.at[r % NSEM]).wait()

    def pump_s(j):
        with scope(f"S{j:02d}"):
            wait_job(sjobs[j], j)
        j2 = j + LOOK
        if j2 < NSJ:
            start_job(sjobs[j2], j2)
        else:
            start_piece(0, 0, j2 - NSJ)

    def pump(h, t, r):
        wait_piece(r)
        r2 = r + LOOK
        if r2 < PPS:
            start_piece(h, t, r2)
        elif t == 0:
            start_piece(h, 1, r2 - PPS)
        else:
            @pl.when(h + 1 < HG)
            def _():
                start_piece(h + 1, 0, r2 - PPS)

            @pl.when(h + 1 == HG)
            def _():
                start_job(ejobs[r2 - PPS], r2 - PPS)

    def pump_e(j):
        with scope(f"E{j:02d}"):
            wait_job(ejobs[j], j)
        j2 = j + LOOK
        if j2 < NEJ:
            start_job(ejobs[j2], j2)

    row = lax.broadcasted_iota(jnp.int32, (B, DH), 0)
    scale = DH ** -0.5

    def qproj(h1, h, j):
        off = (h + j * HG) * DH
        if not isinstance(off, int):
            off = pl.multiple_of(off, DH)
        qbuf[j] = jnp.dot(h1, wq[:, :, pl.ds(off, DH)].reshape(D, DH), preferred_element_type=f32)

    def qk4(c, u, prev):
        j, bh = divmod(u, 2)
        q = qbuf[j].astype(bf16)
        out = prev
        for b in range(4 * bh, 4 * bh + 4):
            sb = lax.dot_general(q, kv[c % NS, NJ * b + j], NT, preferred_element_type=f32)
            out = sb if out is None else jnp.where(row == b, sb, out)
        if bh == 1:
            sbuf[j, c] = out
            return None
        return out

    def pv4(c, u, acc):
        j, bh = divmod(u, 2)
        p = pbuf[j, c]
        for b in range(4 * bh, 4 * bh + 4):
            pb = jnp.where(row == b, p, 0.0).astype(bf16)
            d = jnp.dot(pb, kv[c % NS, NJ * b + j], preferred_element_type=f32)
            acc[j] = d if acc[j] is None else acc[j] + d

    def softmax_max():
        return [jnp.max(functools.reduce(jnp.maximum, [sbuf[j, c] for c in range(NCH)]), axis=-1, keepdims=True)
                for j in range(NJ)]

    def softmax_exp(m):
        for j in range(NJ):
            tot = None
            for c in range(NCH):
                p = jnp.exp((sbuf[j, c] - m[j]) * scale)
                pbuf[j, c] = p
                tot = p if tot is None else tot + p
            linv[j] = jnp.broadcast_to(1.0 / jnp.sum(tot, axis=-1, keepdims=True), (B, DH))

    def pv_last(u, acc, hprev):
        j, bh = divmod(u, 2)
        if bh == 0:
            acc[j] = part[j]
        pv4(NCH - 1, u, acc)
        if bh == 1:
            oacc[hprev + j * HG] = acc[j] * linv[j]

    cc = cpy(c_hbm, cs, xsem.at[0])
    cx = cpy(x_hbm, xs, xsem.at[1])
    cc.start(priority=0)
    cx.start(priority=0)
    for j in range(LOOK):
        start_job(sjobs[j], j)
    pbuf[...] = jnp.zeros_like(pbuf)
    part[...] = jnp.zeros_like(part)
    linv[...] = jnp.zeros_like(linv)
    kv[(NCH - 1) % NS] = jnp.zeros(kv.shape[1:], bf16)
    pump_s(0)
    with scope("cx"):
        cc.wait()
        cx.wait()
    cf = cs[...].astype(f32)
    sc = (cf * jax.nn.sigmoid(cf)).astype(bf16)
    x = xs[...].astype(f32)
    pump_s(1)
    lnx = _ln(x)
    for j in range(2, n_moda):
        pump_s(j)
    moda = jnp.dot(sc, wm[:, :, :2 * D].reshape(D, 2 * D), preferred_element_type=f32)
    pump_s(n_moda)
    h1 = (lnx * (1.0 + moda[:, D:]) + moda[:, :D]).astype(bf16)
    for j in range(n_moda + 1, NSJ):
        pump_s(j)

    def group(h, carry):
        hprev = jnp.where(h > 0, h - 1, H)
        acc = [None] * NJ
        st = None
        for r in range(PPS):
            pump(h, 0, r)
            if not compute:
                continue
            c, u = divmod(r, PPC)
            if c == 0:
                pv_last(u, acc, hprev)
                if u < NJ:
                    qproj(h1, h, u)
            else:
                st = qk4(c - 1, u, st)
        acc = [None] * NJ
        for r in range(PPS):
            pump(h, 1, r)
            if not compute:
                continue
            c, u = divmod(r, PPC)
            if c == 0:
                st = qk4(NCH - 1, u, st)
            elif c == 1:
                if u == 0:
                    m = softmax_max()
                elif u == 1:
                    softmax_exp(m)
                else:
                    pv4(0, 2 * (u - 2), acc)
                    pv4(0, 2 * (u - 2) + 1, acc)
            else:
                pv4(c - 1, u, acc)
        if compute:
            for j in range(NJ):
                part[j] = acc[j]
        return carry

    if not compute:
        oacc[...] = jnp.zeros_like(oacc)
    lax.fori_loop(0, HG, group, 0)

    acc = [None] * NJ
    attn = None
    HPS = H // NW

    def wo_head(hd, attn):
        s_, m_ = divmod(hd, HPS)
        d = jnp.dot(oacc[hd].astype(bf16), wo[s_, pl.ds(m_ * DH, DH), :], preferred_element_type=f32)
        return d if attn is None else attn + d

    for j in range(n_wo):
        pump_e(j)
        if j < PPC and compute:
            pv_last(j, acc, HG - 1)
        if j >= NW:
            attn = wo_head(HPS * (j % NW) + j // NW - 1, attn)
    for j in range(n_m1):
        pump_e(n_wo + j)
        attn = wo_head(HPS * j + HPS - 1, attn)
    pump_e(n_wo + n_m1)
    mod1 = jnp.dot(sc, wm[:, :, 2 * D:4 * D].reshape(D, 2 * D), preferred_element_type=f32)
    pump_e(n_wo + n_m1 + 1)
    x1 = x + mod1[:, :D] * attn
    ln1 = _ln(x1)
    for j in range(n_m1 + 2, 2 * n_m1):
        pump_e(n_wo + j)
    pump_e(g0)
    mod2 = jnp.dot(sc, wm[:, :, 4 * D:].reshape(D, 2 * D), preferred_element_type=f32)
    h2 = (ln1 * (1.0 + mod2[:, :D]) + mod1[:, D:]).astype(bf16)
    y = jnp.zeros((B, D), f32)
    for i, (f0, n) in enumerate(fch):
        if i > 0:
            pump_e(g0 + 3 * i)
        g = lax.dot_general(h2, wg[pl.ds(f0, n), :], NT, preferred_element_type=f32)
        pump_e(g0 + 3 * i + 1)
        u = lax.dot_general(h2, wu[pl.ds(f0, n), :], NT, preferred_element_type=f32)
        a = (jax.nn.sigmoid(g) * u).astype(bf16)
        pump_e(g0 + 3 * i + 2)
        y = y + jnp.dot(a, wd[pl.ds(f0, n), :], preferred_element_type=f32)
    o_ref[...] = (x1 + mod2[:, D:] * y).astype(o_ref.dtype)


@jax.jit
def pallas_adaLN_cond__sliding_block_cached__glu_gated_glu__decode_kernel(A_x, A_k_cache, A_v_cache, A_wq, A_wo, B_x, B_w_gate, B_w_up, B_w_down, c, w_mod):
    S = A_k_cache.shape[2]
    W = min(4096, max(256, S // 4))
    hbm = pl.BlockSpec(memory_space=pltpu.HBM)
    out = pl.pallas_call(
        functools.partial(_body, S=S, W=W, LOOK=8, n0=2, compute=True, scopes=False),
        out_shape=jax.ShapeDtypeStruct((B, D), A_x.dtype),
        in_specs=[hbm] * 10,
        out_specs=pl.BlockSpec(memory_space=pltpu.VMEM),
        scratch_shapes=[
            pltpu.VMEM((NS, NSTR, CH, DH), bf16),
            pltpu.VMEM((B, D), bf16),
            pltpu.VMEM((B, D), bf16),
            pltpu.VMEM((NW, D // NW, 6 * D), bf16),
            pltpu.VMEM((NW, D // NW, H * DH), bf16),
            pltpu.VMEM((NW, H * DH // NW, D), bf16),
            pltpu.VMEM((F, D), bf16),
            pltpu.VMEM((F, D), bf16),
            pltpu.VMEM((F, D), bf16),
            pltpu.VMEM((H + HG + 1, B, DH), f32),
            pltpu.VMEM((NJ, W // CH, B, DH), f32),
            pltpu.VMEM((NJ, W // CH, B, DH), f32),
            pltpu.VMEM((NJ, B, DH), f32),
            pltpu.VMEM((NJ, B, DH), f32),
            pltpu.VMEM((NJ, B, DH), f32),
            pltpu.SemaphoreType.DMA((NSEM,)),
            pltpu.SemaphoreType.DMA((NSEM,)),
            pltpu.SemaphoreType.DMA((2,)),
        ],
        compiler_params=pltpu.CompilerParams(
            vmem_limit_bytes=64 * 1024 * 1024, disable_bounds_checks=True, disable_semaphore_checks=True),
    )(A_x.reshape(B, D), A_k_cache.reshape(NSTR, HG, S, DH), A_v_cache.reshape(NSTR, HG, S, DH),
      A_wq.reshape(NW, D // NW, H * DH), A_wo.reshape(NW, H * DH // NW, D), B_w_gate.T, B_w_up.T, B_w_down, c,
      w_mod.reshape(NW, D // NW, 6 * D))
    return out.reshape(B, 1, D)
```

```python
import functools
import jax
import jax.numpy as jnp
from jax import lax
import jax.experimental.pallas as pl
import jax.experimental.pallas.tpu as pltpu

B, D, H, DH, F = 8, 512, 32, 128, 1376
CH = 128
G = 8
NS = 8
NSEM = 16
NW = 8
NT = (((1,), (1,)), ((), ()))
f32, bf16 = jnp.float32, jnp.bfloat16
cpy = pltpu.make_async_copy


def _ln(x):
    m = jnp.mean(x, axis=-1, keepdims=True)
    d = x - m
    v = jnp.mean(d * d, axis=-1, keepdims=True)
    return d * lax.rsqrt(v + 1e-5)


def _body(x_hbm, k_hbm, v_hbm, wq_hbm, wo_hbm, wg_hbm, wu_hbm, wd_hbm, c_hbm, wm_hbm,
          o_ref,
          kv, xs, cs, wm, wq, wo, wg, wu, wd, oacc, qtab, sbuf, pbuf, part, linv, sems, wsems, xsem,
          *, S, W, LOOK, NJ, compute, scopes):
    NSTR = G * NJ
    R = 64 // NJ
    NG = B * H // NSTR
    n0 = NJ
    NCH = W // CH
    PPC = CH // R
    PPS = NCH * PPC
    assert PPS % NSEM == 0 and NCH % NS == 0 and LOOK <= NSEM and LOOK <= PPC * (NS - 2)
    import contextlib
    scope = (lambda n: jax.named_scope(n)) if scopes else (lambda n: contextlib.nullcontext())

    def rows_job(src, dst, r0, n0_, n, c0=None, nc=None):
        def sl(ref, a, m):
            if c0 is None:
                return ref.at[pl.ds(a, m), :]
            return ref.at[pl.ds(a, m), pl.ds(c0, nc)]
        return [(sl(src, r0, n0_), sl(dst, r0, n0_), 0), (sl(src, r0 + n0_, n - n0_), sl(dst, r0 + n0_, n - n0_), 1)]

    def strm_job(src, dst, r0, nr, c0, nc):
        def sl(ref, a, n):
            return ref.at[pl.ds(a, n), pl.ds(r0, nr), pl.ds(c0, nc)]
        return [(sl(src, 0, 1), sl(dst, 0, 1), 0), (sl(src, 1, NW - 1), sl(dst, 1, NW - 1), 1)]

    def wm_jobs(cb):
        return [strm_job(wm_hbm, wm, 8 * j, 8, 2 * D * cb, 2 * D) for j in range(D // NW // 8)]

    sjobs = wm_jobs(0)
    n_moda = len(sjobs)
    sjobs += [strm_job(wq_hbm, wq, 8 * rb, 8, 1024 * cb, 1024) for cb in range(H * DH // 1024) for rb in range(D // NW // 8)]
    sjobs += wm_jobs(1)
    NSJ = len(sjobs)
    ejobs = [strm_job(wo_hbm, wo, 16 * j, 16, 0, D) for j in range(H * DH // NW // 16)]
    n_wo = len(ejobs)
    ejobs += wm_jobs(2)
    g0 = len(ejobs)
    n_m1 = g0 - n_wo
    fch = [(128 * j, min(128, F - 128 * j)) for j in range(-(-F // 128))]
    for f0, n in fch:
        ejobs += [rows_job(wg_hbm, wg, f0, 16, n), rows_job(wu_hbm, wu, f0, 16, n), rows_job(wd_hbm, wd, f0, 16, n)]
    NEJ = len(ejobs)

    def start_job(job, g):
        for src, dst, prio in sorted(job, key=lambda t: -t[2]):
            cpy(src, dst, wsems.at[g % NSEM]).start(priority=prio)

    def wait_job(job, g):
        for src, dst, prio in job:
            cpy(src, dst, wsems.at[g % NSEM]).wait()

    def start_piece(h, t, r):
        c, pc = divmod(r, PPC)
        rows = pl.ds(S - W + r * R, R)
        dst = pl.ds(pc * R, R)
        src = (k_hbm, v_hbm)[t]
        sem = sems.at[r % NSEM]
        cpy(src.at[h, pl.ds(n0, NSTR - n0), rows, :], kv.at[c % NS, pl.ds(n0, NSTR - n0), dst], sem).start(priority=1)
        cpy(src.at[h, pl.ds(0, n0), rows, :], kv.at[c % NS, pl.ds(0, n0), dst], sem).start(priority=0)

    def wait_piece(r):
        c, pc = divmod(r, PPC)
        dst = kv.at[c % NS, :, pl.ds(pc * R, R)]
        cpy(dst, dst, sems.at[r % NSEM]).wait()

    def pump_s(j):
        with scope(f"S{j:02d}"):
            wait_job(sjobs[j], j)
        j2 = j + LOOK
        if j2 < NSJ:
            start_job(sjobs[j2], j2)
        else:
            start_piece(0, 0, j2 - NSJ)

    def pump(h, t, r):
        wait_piece(r)
        r2 = r + LOOK
        if r2 < PPS:
            start_piece(h, t, r2)
        elif t == 0:
            start_piece(h, 1, r2 - PPS)
        else:
            @pl.when(h + 1 < NG)
            def _():
                start_piece(h + 1, 0, r2 - PPS)

            @pl.when(h + 1 == NG)
            def _():
                start_job(ejobs[r2 - PPS], r2 - PPS)

    def pump_e(j):
        with scope(f"E{j:02d}"):
            wait_job(ejobs[j], j)
        j2 = j + LOOK
        if j2 < NEJ:
            start_job(ejobs[j2], j2)

    row = lax.broadcasted_iota(jnp.int32, (B, DH), 0)
    scale = DH ** -0.5

    def qproj(h1, hd):
        q = jnp.dot(h1, wq[:, :, pl.ds(hd * DH, DH)].reshape(D, DH), preferred_element_type=f32)
        qtab[pl.ds(hd, B, stride=H), :] = q

    def rows8(g, j):
        return pl.ds(pl.multiple_of(g * NSTR + j * G, G), G)

    def qk4(g, c, u, prev):
        j, bh = divmod(u, 2)
        q = qtab[rows8(g, j), :].astype(bf16)
        out = prev
        for b in range(4 * bh, 4 * bh + 4):
            sb = lax.dot_general(q, kv[c % NS, G * j + b], NT, preferred_element_type=f32)
            out = sb if out is None else jnp.where(row == b, sb, out)
        if bh == 1:
            sbuf[j, c] = out
            return None
        return out

    def pv4(c, u, acc):
        j, bh = divmod(u, 2)
        p = pbuf[j, c]
        for b in range(4 * bh, 4 * bh + 4):
            pb = jnp.where(row == b, p, 0.0).astype(bf16)
            d = jnp.dot(pb, kv[c % NS, G * j + b], preferred_element_type=f32)
            acc[j] = d if acc[j] is None else acc[j] + d

    def softmax_max():
        return [jnp.max(functools.reduce(jnp.maximum, [sbuf[j, c] for c in range(NCH)]), axis=-1, keepdims=True)
                for j in range(NJ)]

    def softmax_exp(m):
        for j in range(NJ):
            tot = None
            for c in range(NCH):
                p = jnp.exp((sbuf[j, c] - m[j]) * scale)
                pbuf[j, c] = p
                tot = p if tot is None else tot + p
            linv[j] = jnp.broadcast_to(1.0 / jnp.sum(tot, axis=-1, keepdims=True), (B, DH))

    def pv_last(u, acc, hprev):
        j, bh = divmod(u, 2)
        if bh == 0:
            acc[j] = part[j]
        pv4(NCH - 1, u, acc)
        if bh == 1:
            oacc[rows8(hprev, j), :] = acc[j] * linv[j]

    cc = cpy(c_hbm, cs, xsem.at[0])
    cx = cpy(x_hbm, xs, xsem.at[1])
    cc.start(priority=0)
    cx.start(priority=0)
    for j in range(LOOK):
        start_job(sjobs[j], j)
    pbuf[...] = jnp.zeros_like(pbuf)
    part[...] = jnp.zeros_like(part)
    linv[...] = jnp.zeros_like(linv)
    kv[(NCH - 1) % NS] = jnp.zeros(kv.shape[1:], bf16)
    pump_s(0)
    with scope("cx"):
        cc.wait()
        cx.wait()
    cf = cs[...].astype(f32)
    sc = (cf * jax.nn.sigmoid(cf)).astype(bf16)
    x = xs[...].astype(f32)
    pump_s(1)
    lnx = _ln(x)
    for j in range(2, n_moda):
        pump_s(j)
    moda = jnp.dot(sc, wm[:, :, :2 * D].reshape(D, 2 * D), preferred_element_type=f32)
    pump_s(n_moda)
    h1 = (lnx * (1.0 + moda[:, D:]) + moda[:, :D]).astype(bf16)
    for j in range(n_moda + 1, NSJ):
        pump_s(j)
        if j >= 2 * n_moda and compute:
            qproj(h1, j - 2 * n_moda)

    def group(h, carry):
        hprev = jnp.where(h > 0, h - 1, NG)
        acc = [None] * NJ
        st = None
        for r in range(PPS):
            pump(h, 0, r)
            if not compute:
                continue
            c, u = divmod(r, PPC)
            if c == 0:
                pv_last(u, acc, hprev)
            else:
                st = qk4(h, c - 1, u, st)
        acc = [None] * NJ
        done = 0
        for r in range(PPS):
            pump(h, 1, r)
            if not compute:
                continue
            c, u = divmod(r, PPC)
            if c == 0:
                st = qk4(h, NCH - 1, u, st)
            elif r == PPC:
                m = softmax_max()
            elif r == PPC + 1:
                softmax_exp(m)
            else:
                todo = min(2, c * PPC + (u + 1) - PPC - done, (NCH - 1) * PPC - done)
                todo = min(todo, c * PPC - done)
                for _ in range(todo):
                    pv4(done // PPC, done % PPC, acc)
                    done += 1
        if compute:
            assert done == (NCH - 1) * PPC
            for j in range(NJ):
                part[j] = acc[j]
        return carry

    if not compute:
        oacc[...] = jnp.zeros_like(oacc)
    lax.fori_loop(0, NG, group, 0)

    acc = [None] * NJ
    attn = None
    HPS = H // NW

    def wo_head(hd, attn):
        s_, m_ = divmod(hd, HPS)
        d = jnp.dot(oacc[pl.ds(hd, B, stride=H), :].astype(bf16), wo[s_, pl.ds(m_ * DH, DH), :], preferred_element_type=f32)
        return d if attn is None else attn + d

    for j in range(n_wo):
        pump_e(j)
        if j < PPC and compute:
            pv_last(j, acc, NG - 1)
        if j == 4:
            ga = jnp.dot(sc, wm[:, :, 2 * D:3 * D].reshape(D, D), preferred_element_type=f32)
        if j == 5:
            sb = jnp.dot(sc, wm[:, :, 3 * D:4 * D].reshape(D, D), preferred_element_type=f32)
        if j >= NW:
            attn = wo_head(HPS * (j % NW) + j // NW - 1, attn)
    for j in range(n_m1):
        pump_e(n_wo + j)
        attn = wo_head(HPS * j + HPS - 1, attn)
    pump_e(g0)
    x1 = x + ga * attn
    mod2 = jnp.dot(sc, wm[:, :, 4 * D:].reshape(D, 2 * D), preferred_element_type=f32)
    h2 = (_ln(x1) * (1.0 + mod2[:, :D]) + sb).astype(bf16)
    y = jnp.zeros((B, D), f32)
    for i, (f0, n) in enumerate(fch):
        if i > 0:
            pump_e(g0 + 3 * i)
        g = lax.dot_general(h2, wg[pl.ds(f0, n), :], NT, preferred_element_type=f32)
        pump_e(g0 + 3 * i + 1)
        u = lax.dot_general(h2, wu[pl.ds(f0, n), :], NT, preferred_element_type=f32)
        a = (jax.nn.sigmoid(g) * u).astype(bf16)
        pump_e(g0 + 3 * i + 2)
        y = y + jnp.dot(a, wd[pl.ds(f0, n), :], preferred_element_type=f32)
    o_ref[...] = (x1 + mod2[:, D:] * y).astype(o_ref.dtype)


@jax.jit
def pallas_adaLN_cond__sliding_block_cached__glu_gated_glu__decode_kernel(A_x, A_k_cache, A_v_cache, A_wq, A_wo, B_x, B_w_gate, B_w_up, B_w_down, c, w_mod):
    del B_x
    LOOK = 8
    NJ = 1
    compute = True
    scopes = False
    NSTR = G * NJ
    NG = B * H // NSTR
    S = A_k_cache.shape[2]
    W = min(4096, max(256, S // 4))
    hbm = pl.BlockSpec(memory_space=pltpu.HBM)
    out = pl.pallas_call(
        functools.partial(_body, S=S, W=W, LOOK=LOOK, NJ=NJ, compute=compute, scopes=scopes),
        out_shape=jax.ShapeDtypeStruct((B, D), A_x.dtype),
        in_specs=[hbm] * 10,
        out_specs=pl.BlockSpec(memory_space=pltpu.VMEM),
        scratch_shapes=[
            pltpu.VMEM((NS, NSTR, CH, DH), bf16),
            pltpu.VMEM((B, D), bf16),
            pltpu.VMEM((B, D), bf16),
            pltpu.VMEM((NW, D // NW, 6 * D), bf16),
            pltpu.VMEM((NW, D // NW, H * DH), bf16),
            pltpu.VMEM((NW, H * DH // NW, D), bf16),
            pltpu.VMEM((F, D), bf16),
            pltpu.VMEM((F, D), bf16),
            pltpu.VMEM((F, D), bf16),
            pltpu.VMEM(((NG + 1) * NSTR, DH), f32),
            pltpu.VMEM((B * H, DH), f32),
            pltpu.VMEM((NJ, W // CH, B, DH), f32),
            pltpu.VMEM((NJ, W // CH, B, DH), f32),
            pltpu.VMEM((NJ, B, DH), f32),
            pltpu.VMEM((NJ, B, DH), f32),
            pltpu.SemaphoreType.DMA((NSEM,)),
            pltpu.SemaphoreType.DMA((NSEM,)),
            pltpu.SemaphoreType.DMA((2,)),
        ],
        compiler_params=pltpu.CompilerParams(
            vmem_limit_bytes=64 * 1024 * 1024, disable_bounds_checks=True, disable_semaphore_checks=True),
    )(A_x.reshape(B, D), A_k_cache.reshape(NG, NSTR, S, DH), A_v_cache.reshape(NG, NSTR, S, DH),
      A_wq.reshape(NW, D // NW, H * DH), A_wo.reshape(NW, H * DH // NW, D), B_w_gate.T, B_w_up.T, B_w_down, c,
      w_mod.reshape(NW, D // NW, 6 * D))
    return out.reshape(B, 1, D)
```

```python
import functools

import jax
import jax.numpy as jnp
from jax import lax
import jax.experimental.pallas as pl
import jax.experimental.pallas.tpu as pltpu

B, D, H, DH, F = 8, 512, 32, 128, 1376
G = 8
CH = 128
R = 64
PPC = CH // R
NS = 8
NW = 8
LOOK = 8
NSEM = 16
NT = (((1,), (1,)), ((), ()))
f32, bf16 = jnp.float32, jnp.bfloat16
cpy = pltpu.make_async_copy


def _kernel(x_hbm, k_hbm, v_hbm, wq_hbm, wo_hbm, wg_hbm, wu_hbm, wd_hbm, c_hbm, wm_hbm,
            o_ref,
            kv, xs, cs, wm, wq, wo, wg, wu, wd,
            otab, qtab, modb, attn, sbuf, pbuf, part, linv,
            sems, wsems, xsem, *, S, W):
    NHG = H // G
    NG = B * NHG
    NCH = W // CH
    PPS = NCH * PPC
    assert PPS % NSEM == 0 and NCH % NS == 0 and LOOK <= min(NSEM, PPC * (NS - 2))

    def rows_job(src, dst, r0, n):
        return [(src.at[pl.ds(r0 + 16, n - 16)], dst.at[pl.ds(r0 + 16, n - 16)], 1),
                (src.at[pl.ds(r0, 16)], dst.at[pl.ds(r0, 16)], 0)]

    def strm_job(src, dst, r0, nr, c0, nc):
        def sl(ref, a, n):
            return ref.at[pl.ds(a, n), pl.ds(r0, nr), pl.ds(c0, nc)]
        return [(sl(src, 1, NW - 1), sl(dst, 1, NW - 1), 1), (sl(src, 0, 1), sl(dst, 0, 1), 0)]

    NRB = D // NW // 8
    sjobs = [strm_job(wm_hbm, wm, 8 * rb, 8, 1024 * cb, 1024)
             for rb in range(NRB) for cb in range(6 * D // 1024)]
    n_wm = len(sjobs)
    sjobs += [strm_job(wq_hbm, wq, 8 * rb, 8, 1024 * cb, 1024)
              for rb in range(NRB) for cb in range(H * DH // 1024)]
    n_wq = len(sjobs)
    sjobs += [strm_job(wo_hbm, wo, 16 * j, 16, 0, D) for j in range(H * DH // NW // 16)]
    NSJ = len(sjobs)

    offs, lens = (0, 464, 928), (464, 464, 448)
    assert offs[2] + lens[2] == F
    ejobs = []
    for i in range(max(lens) // 16):
        job = [(src.at[pl.ds(offs[t] + 16 * i, 16)], dst.at[pl.ds(offs[t] + 16 * i, 16)], 1)
               for t in range(3) if 16 * i < lens[t] for src, dst in ((wu_hbm, wu), (wg_hbm, wg))][1:]
        job += [(wu_hbm.at[pl.ds(16 * i, 16)], wu.at[pl.ds(16 * i, 16)], 0)]
        ejobs.append(job)
    n_gu = len(ejobs)
    units = [(offs[t] + 128 * w, min(128, lens[t] - 128 * w)) for w in range(4) for t in range(3)]
    yord = [0, 1, 2, 9, 10, 11, 3, 4, 5, 6, 7, 8]
    ejobs += [rows_job(wd_hbm, wd, *units[k]) for k in yord]
    NEJ = len(ejobs)

    def start_job(jobs, j):
        for src, dst, q in jobs[j]:
            cpy(src, dst, wsems.at[j % NSEM]).start(priority=q)

    def wait_job(jobs, j):
        for src, dst, _ in jobs[j]:
            cpy(src, dst, wsems.at[j % NSEM]).wait()

    def kv_group(gi):
        return (gi % B) * NHG + gi // B

    def start_piece(gi, t, r):
        c, pc = divmod(r, PPC)
        rows = pl.ds(S - W + r * R, R)
        dst = pl.ds(pc * R, R)
        src = (k_hbm, v_hbm)[t]
        g = kv_group(gi)
        sem = sems.at[r % NSEM]
        cpy(src.at[g, pl.ds(1, G - 1), rows, :], kv.at[c % NS, pl.ds(1, G - 1), dst], sem).start(priority=1)
        cpy(src.at[g, pl.ds(0, 1), rows, :], kv.at[c % NS, pl.ds(0, 1), dst], sem).start(priority=0)

    def wait_piece(r):
        c, pc = divmod(r, PPC)
        dst = kv.at[c % NS, :, pl.ds(pc * R, R)]
        cpy(dst, dst, sems.at[r % NSEM]).wait()

    def pump_s(j):
        wait_job(sjobs, j)
        if j + LOOK < NSJ:
            start_job(sjobs, j + LOOK)
        else:
            start_piece(0, 0, j + LOOK - NSJ)

    def pump(gi, t, r):
        wait_piece(r)
        r2 = r + LOOK
        if r2 < PPS:
            start_piece(gi, t, r2)
        elif t == 0:
            start_piece(gi, 1, r2 - PPS)
        else:
            @pl.when(gi + 1 < NG)
            def _():
                start_piece(gi + 1, 0, r2 - PPS)

            @pl.when(gi + 1 == NG)
            def _():
                start_job(ejobs, r2 - PPS)

    def pump_e(j):
        wait_job(ejobs, j)
        if j + LOOK < NEJ:
            start_job(ejobs, j + LOOK)

    row = lax.broadcasted_iota(jnp.int32, (G, DH), 0)
    scale = DH ** -0.5

    def rows8(g):
        return pl.ds(pl.multiple_of(g * G, G), G)

    def qk4(gi, c, u, prev):
        q = qtab[rows8(kv_group(gi)), :].astype(bf16)
        out = prev
        for hh in range(4 * u, 4 * u + 4):
            s = lax.dot_general(q, kv[c % NS, hh], NT, preferred_element_type=f32)
            out = s if out is None else jnp.where(row == hh, s, out)
        if u == PPC - 1:
            sbuf[c] = out
            return None
        return out

    def pv4(c, u, acc):
        p = pbuf[c]
        for hh in range(4 * u, 4 * u + 4):
            ph = jnp.where(row == hh, p, 0.0).astype(bf16)
            d = jnp.dot(ph, kv[c % NS, hh], preferred_element_type=f32)
            acc = d if acc is None else acc + d
        return acc

    def pv_last(u, acc, g):
        if u == 0:
            acc = part[...]
        acc = pv4(NCH - 1, u, acc)
        if u == PPC - 1:
            otab[rows8(g), :] = acc * linv[...]
        return acc

    def wo_head(hd):
        s_, m_ = hd // (H // NW), (hd % (H // NW)) * DH
        if not isinstance(hd, int):
            m_ = pl.multiple_of(m_, DH)
        return jnp.dot(otab[pl.ds(hd, B, stride=H), :].astype(bf16), wo[s_, pl.ds(m_, DH), :],
                       preferred_element_type=f32)

    cc = cpy(c_hbm, cs, xsem.at[0])
    cx = cpy(x_hbm, xs, xsem.at[1])
    cc.start(priority=0)
    cx.start(priority=0)
    for j in range(LOOK):
        start_job(sjobs, j)
    pbuf[...] = jnp.zeros_like(pbuf)
    part[...] = jnp.zeros_like(part)
    linv[...] = jnp.zeros_like(linv)
    kv[(NCH - 1) % NS] = jnp.zeros(kv.shape[1:], bf16)
    otab[...] = jnp.zeros_like(otab)
    attn[...] = jnp.zeros_like(attn)

    pump_s(0)
    cc.wait()
    cx.wait()
    cf = cs[...].astype(f32)
    sc = (cf * jax.nn.sigmoid(cf)).astype(bf16)
    x = xs[...].astype(f32)
    xd = x - jnp.mean(x, axis=-1, keepdims=True)
    pump_s(1)
    xv = jnp.mean(xd * xd, axis=-1, keepdims=True)
    pump_s(2)
    lnx = xd * lax.rsqrt(xv + 1e-5)
    for j in range(3, n_wm):
        pump_s(j)

    ma = []
    for j in range(n_wm, n_wq):
        pump_s(j)
        t = j - n_wm
        if t < 24:
            m = jnp.dot(sc, wm[:, :, pl.ds(t * DH, DH)].reshape(D, DH), preferred_element_type=f32)
            if t < 8:
                ma.append(m)
            else:
                modb[t - 8] = m
        if t == 8:
            h1 = (lnx * (1.0 + jnp.concatenate(ma[4:], axis=1)) + jnp.concatenate(ma[:4], axis=1)).astype(bf16)

    for j in range(n_wq, NSJ):
        pump_s(j)
        hd = j - n_wq
        qtab[pl.ds(hd, B, stride=H), :] = jnp.dot(
            h1, wq[:, :, pl.ds(hd * DH, DH)].reshape(D, DH), preferred_element_type=f32)

    def group(gi, carry):
        gprev = jnp.where(gi > 0, kv_group(gi - 1), NG)
        acc = st = None
        for r in range(PPS):
            pump(gi, 0, r)
            c, u = divmod(r, PPC)
            if c == 0:
                acc = pv_last(u, acc, gprev)
            else:
                st = qk4(gi, c - 1, u, st)
        acc = None
        done = 0
        for r in range(PPS):
            pump(gi, 1, r)
            c, u = divmod(r, PPC)
            if c == 0:
                st = qk4(gi, NCH - 1, u, st)
            elif r == PPC:
                mx = jnp.max(functools.reduce(jnp.maximum, [sbuf[i] for i in range(NCH)]),
                             axis=-1, keepdims=True)
                hd = gi - (B + 1)
                attn[...] += jnp.where(hd >= 0, wo_head(jnp.maximum(hd, 0)), 0.0)
            elif r == PPC + 1:
                tot = None
                for i in range(NCH):
                    p = jnp.exp((sbuf[i] - mx) * scale)
                    pbuf[i] = p
                    tot = p if tot is None else tot + p
                linv[...] = jnp.broadcast_to(1.0 / jnp.sum(tot, axis=-1, keepdims=True), (G, DH))
            else:
                for _ in range(min(2, r - PPC - done + 1, (NCH - 1) * PPC - done, c * PPC - done)):
                    acc = pv4(done // PPC, done % PPC, acc)
                    done += 1
        assert done == (NCH - 1) * PPC
        part[...] = acc
        return carry

    lax.fori_loop(0, NG, group, 0)

    def mod(i):
        return jnp.concatenate([modb[4 * i + k] for k in range(4)], axis=1)

    hd0 = NG - (B + 1)
    acc = a = h2 = None
    acts = {}
    y = jnp.zeros((B, D), f32)
    for j in range(NEJ):
        pump_e(j)
        if j < PPC:
            acc = pv_last(j, acc, kv_group(NG - 1))
        elif j < PPC + 5:
            k = j - PPC
            if k == 0:
                a = attn[...]
            for hd in range(hd0 + 2 * k, min(hd0 + 2 * k + 2, H)):
                a = a + wo_head(hd)
        elif j == PPC + 5:
            x1 = x + mod(0) * a
            xd = x1 - jnp.mean(x1, axis=-1, keepdims=True)
        elif j == PPC + 6:
            xv = jnp.mean(xd * xd, axis=-1, keepdims=True)
        elif j == PPC + 7:
            h2 = (xd * lax.rsqrt(xv + 1e-5) * (1.0 + mod(2)) + mod(1)).astype(bf16)
        else:
            avail = 3 * min((j + 1) // 8, 3) + (3 if j >= n_gu - 1 else 0)
            if len(acts) < avail:
                f0, n = units[len(acts)]
                g = lax.dot_general(h2, wg[pl.ds(f0, n), :], NT, preferred_element_type=f32)
                up = lax.dot_general(h2, wu[pl.ds(f0, n), :], NT, preferred_element_type=f32)
                acts[len(acts)] = (jax.nn.sigmoid(g) * up).astype(bf16)
            if j >= n_gu:
                k = yord[j - n_gu]
                f0, n = units[k]
                y = y + jnp.dot(acts[k], wd[pl.ds(f0, n), :], preferred_element_type=f32)
    o_ref[...] = (x1 + mod(3) * y).astype(o_ref.dtype)


@jax.jit
def pallas_adaLN_cond__sliding_block_cached__glu_gated_glu__decode_kernel(
    A_x, A_k_cache, A_v_cache, A_wq, A_wo, B_x, B_w_gate, B_w_up, B_w_down, c, w_mod,
):
    del B_x
    S = A_k_cache.shape[2]
    W = min(4096, max(256, S // 4))
    NG = B * H // G
    hbm = pl.BlockSpec(memory_space=pltpu.HBM)
    out = pl.pallas_call(
        functools.partial(_kernel, S=S, W=W),
        out_shape=jax.ShapeDtypeStruct((B, D), A_x.dtype),
        in_specs=[hbm] * 10,
        out_specs=pl.BlockSpec(memory_space=pltpu.VMEM),
        scratch_shapes=[
            pltpu.VMEM((NS, G, CH, DH), bf16),
            pltpu.VMEM((B, D), bf16),
            pltpu.VMEM((B, D), bf16),
            pltpu.VMEM((NW, D // NW, 6 * D), bf16),
            pltpu.VMEM((NW, D // NW, H * DH), bf16),
            pltpu.VMEM((NW, H * DH // NW, D), bf16),
            pltpu.VMEM((F, D), bf16),
            pltpu.VMEM((F, D), bf16),
            pltpu.VMEM((F, D), bf16),
            pltpu.VMEM(((B + 1) * H, DH), f32),
            pltpu.VMEM(((B + 1) * H, DH), f32),
            pltpu.VMEM((16, B, DH), f32),
            pltpu.VMEM((B, D), f32),
            pltpu.VMEM((W // CH, G, DH), f32),
            pltpu.VMEM((W // CH, G, DH), f32),
            pltpu.VMEM((G, DH), f32),
            pltpu.VMEM((G, DH), f32),
            pltpu.SemaphoreType.DMA((NSEM,)),
            pltpu.SemaphoreType.DMA((NSEM,)),
            pltpu.SemaphoreType.DMA((2,)),
        ],
        compiler_params=pltpu.CompilerParams(
            vmem_limit_bytes=64 * 1024 * 1024, disable_semaphore_checks=True),
    )(A_x.reshape(B, D), A_k_cache.reshape(NG, G, S, DH), A_v_cache.reshape(NG, G, S, DH),
      A_wq.reshape(NW, D // NW, H * DH), A_wo.reshape(NW, H * DH // NW, D),
      B_w_gate.T, B_w_up.T, B_w_down, c, w_mod.reshape(NW, D // NW, 6 * D))
    return out.reshape(B, 1, D)
```
